```python
import jax
import jax.numpy as jnp

def _softmax(x, axis=-1):
    return jax.nn.softmax(x, axis=axis)
def _gelu(x):
    return jax.nn.gelu(x, approximate=True)
def _silu(x):
    return jax.nn.silu(x)
def _sigmoid(x):
    return jax.nn.sigmoid(x)
def _layernorm(x, axis=-1, eps=1e-5):
    m = jnp.mean(x, axis=axis, keepdims=True)
    v = jnp.var(x, axis=axis, keepdims=True)
    return (x - m) / jnp.sqrt(v + eps)
def _scatter_add(tgt, idx, src, axis=0):
    return tgt.at[idx].add(src)
def _segment_sum(src, seg, n):
    return jax.ops.segment_sum(src, seg, n)
class _Rng:
    def __init__(self, key):
        self._k = key
    def _next(self):
        self._k, sub = jax.random.split(self._k)
        return sub
    def normal(self, shape):
        return jax.random.normal(self._next(), shape, dtype=jnp.bfloat16)
    def randint(self, lo, hi, shape):
        return jax.random.randint(self._next(), shape, lo, hi, dtype=jnp.int32)
    def uniform(self, shape, lo=0.0, hi=1.0):
        return jax.random.uniform(self._next(), shape, jnp.bfloat16, lo, hi)
    def permutation(self, n):
        return jax.random.permutation(self._next(), n)


kernel_name = 'standalone__layerscale__sampling'

def _fwd_setup_inputs():
    _rng = _Rng(jax.random.key(int.from_bytes(__import__("os").urandom(4), "little")))
    _w = (lambda a: (lambda t: t.astype(jnp.bfloat16) if jnp.issubdtype(t.dtype, jnp.floating) else t)(jnp.asarray(a)))
    B, S, D = 1024, 8, 512
    return {
        "x": _w((lambda *s: _rng.normal(s) * 0.05)(B, S, D)),
        "y": _w((lambda *s: _rng.normal(s) * 0.05)(B, S, D)),
        "gamma": _w(1e-4 * (lambda *s: _rng.normal(s) * 0.05)(D)),
    }

def _fwd_reference(x, y, gamma):
    return x + gamma * y


def setup_inputs():
    _inp = _fwd_setup_inputs()
    _gk = jax.random.fold_in(jax.random.key(int.from_bytes(__import__("os").urandom(4), "little")), 2**31 - 1)
    _shapes = [[1024, 8, 512]]
    _dtypes = ['bfloat16']
    _gks = jax.random.split(_gk, len(_shapes))
    _gs = [jax.random.normal(k, s, dtype=jnp.dtype(d)) * 0.05 for k, s, d in zip(_gks, _shapes, _dtypes)]
    _inp["grad_out"] = _gs[0]
    return _inp

def reference(x, y, gamma, grad_out):
    _const = dict()
    def _f(*_d):
        return _fwd_reference(**{'x': _d[0], 'y': _d[1], 'gamma': _d[2], **_const})
    _out, _vjp = jax.vjp(_f, x, y, gamma)
    _grads = _vjp(grad_out)
    _out0 = jnp.asarray(_out)
    return (_out0, *[jnp.asarray(_g) for _g in _grads])
```

```python
import jax
import jax.numpy as jnp
import jax.experimental.pallas as pl
import jax.experimental.pallas.tpu as pltpu


_GROUPS = 8
_KR = 24
_KW = 16
_TAIL = 48
_P = 32
_Q = 88
_XSPLIT = 384
_SUB = 16


@jax.jit
def pallas_standalone__layerscale__sampling_kernel(
    x: jax.Array,
    y: jax.Array,
    gamma: jax.Array,
    grad_out: jax.Array,
):
    B, S, D = x.shape
    G = _GROUPS
    RG = (B * S) // G
    A = RG - 2 * _P - _Q
    B1 = (A + _P) // _KW * _KW
    f32 = jnp.float32

    def kernel_function(x_hbm, y_hbm, gam_hbm, g_hbm, o_hbm, gx_hbm, gy_hbm, gg_hbm,
                        xb, yb, gb, gyb, gamb, ggb, smp, smq, sems):
        def copy_rows(src, dst, sem, lo, n):
            return pltpu.make_async_copy(
                src.at[:, pl.ds(lo, n)], dst.at[:, pl.ds(lo, n)], sem)

        def start_rows(src, dst, sem, k, lo, hi):
            n = (hi - lo) // k

            def step(j, carry):
                copy_rows(src, dst, sem, pl.multiple_of(lo + j * k, 8), k).start()
                return carry
            jax.lax.fori_loop(0, n, step, 0)
            if lo + n * k < hi:
                copy_rows(src, dst, sem, lo + n * k, hi - lo - n * k).start()

        def wait_rows(src, dst, sem, lo, hi):
            copy_rows(src, dst, sem, lo, hi - lo).wait()

        def row_loop(body, init, lo, hi):
            def step(i, carry):
                r = pl.ds(pl.multiple_of(lo + i * _SUB, _SUB), _SUB)
                for gi in range(G):
                    carry = body(gi, r, carry)
                return carry
            return jax.lax.fori_loop(0, (hi - lo) // _SUB, step, init)

        s_g, s_gam, s_y, s_x, s_xt, s_p, s_q, s_gx, s_gy, s_o, s_gg = (
            sems.at[i] for i in range(11))
        p1, q0, p2 = A, A + _P, A + _P + _Q
        p1_in = pltpu.make_async_copy(x_hbm.at[:, pl.ds(p1, _P)], smp, s_p)
        p1_fwd = pltpu.make_async_copy(smp, xb.at[:, pl.ds(p1, _P)], s_p)
        p2_in = pltpu.make_async_copy(x_hbm.at[:, pl.ds(p2, _P)], smp, s_p)
        p2_fwd = pltpu.make_async_copy(smp, xb.at[:, pl.ds(p2, _P)], s_p)
        q_in = pltpu.make_async_copy(x_hbm.at[:, pl.ds(q0, _Q)], smq, s_q)
        q_fwd = pltpu.make_async_copy(smq, xb.at[:, pl.ds(q0, _Q)], s_q)
        gam_in = pltpu.make_async_copy(gam_hbm, gamb, s_gam)
        gg_out = pltpu.make_async_copy(ggb, gg_hbm, s_gg)

        copy_rows(g_hbm, gb, s_g, 0, _KR).start()
        p1_in.start()
        q_in.start()
        gam_in.start()
        start_rows(g_hbm, gb, s_g, _KR, _KR, RG)
        p1_in.wait()
        p1_fwd.start()
        start_rows(y_hbm, yb, s_y, _KR, 0, RG)
        start_rows(x_hbm, xb, s_x, _KR, 0, _XSPLIT)
        p1_fwd.wait()
        p2_in.start()
        start_rows(x_hbm, xb, s_x, _KR, _XSPLIT, A - _TAIL)
        start_rows(x_hbm, xb, s_xt, _KR, A - _TAIL, A)

        wait_rows(g_hbm, gb, s_g, 0, RG)
        gam_in.wait()
        gam = jnp.broadcast_to(gamb[...].astype(f32).reshape(1, D), (_SUB, D))

        def grad_y_step(gi, r, carry):
            gyb[gi, r, :] = (gam * gb[gi, r, :].astype(f32)).astype(gyb.dtype)
            return carry
        row_loop(grad_y_step, 0, 0, RG)

        wait_rows(y_hbm, yb, s_y, 0, RG)

        def grad_gamma_step(gi, r, acc):
            prod = gb[gi, r, :].astype(f32) * yb[gi, r, :].astype(f32)
            return acc + prod.reshape(_SUB // 8, 8, D).sum(axis=0)
        acc = row_loop(grad_gamma_step, jnp.zeros((8, D), f32), 0, RG)
        ggb[...] = jnp.sum(acc, axis=0).astype(ggb.dtype)

        wait_rows(x_hbm, xb, s_x, 0, A - _TAIL)
        start_rows(gb, gx_hbm, s_gx, _KW, 0, RG)
        q_in.wait()
        p2_in.wait()
        q_fwd.start()
        p2_fwd.start()
        gg_out.start()
        wait_rows(x_hbm, xb, s_xt, A - _TAIL, A)

        def out_step(gi, r, carry):
            xb[gi, r, :] = (xb[gi, r, :].astype(f32)
                            + gam * yb[gi, r, :].astype(f32)).astype(xb.dtype)
            return carry
        row_loop(out_step, 0, 0, B1)
        start_rows(gyb, gy_hbm, s_gy, _KW, 0, RG)
        start_rows(xb, o_hbm, s_o, _KW, 0, B1)
        q_fwd.wait()
        p2_fwd.wait()
        row_loop(out_step, 0, B1, RG)
        start_rows(xb, o_hbm, s_o, _KW, B1, RG)

        wait_rows(gb, gx_hbm, s_gx, 0, RG)
        gg_out.wait()
        wait_rows(gyb, gy_hbm, s_gy, 0, RG)
        wait_rows(xb, o_hbm, s_o, 0, RG)

    shp = (G, RG, D)
    any_spec = pl.BlockSpec(memory_space=pl.ANY)
    big = jax.ShapeDtypeStruct(shp, x.dtype)
    out, gx, gy, gg = pl.pallas_call(
        kernel_function,
        in_specs=[any_spec] * 4,
        out_specs=[any_spec] * 4,
        out_shape=[big, big, big, jax.ShapeDtypeStruct((D,), gamma.dtype)],
        scratch_shapes=[pltpu.VMEM(shp, x.dtype)] * 4
        + [pltpu.VMEM((D,), gamma.dtype)] * 2
        + [pltpu.SMEM((G, _P, D), x.dtype), pltpu.SMEM((G, _Q, D), x.dtype)]
        + [pltpu.SemaphoreType.DMA((11,))],
        compiler_params=pltpu.CompilerParams(
            vmem_limit_bytes=48 * 1024 * 1024, disable_semaphore_checks=True),
    )(x.reshape(shp), y.reshape(shp), gamma, grad_out.reshape(shp))
    return out.reshape(B, S, D), gx.reshape(B, S, D), gy.reshape(B, S, D), gg
```

```python
import jax
import jax.numpy as jnp
import jax.experimental.pallas as pl
import jax.experimental.pallas.tpu as pltpu


_G = 8
_NLO = 2
_KR = 24
_KG = 32
_KW = 16
_P = 32
_Q = 136
_FWD_EVERY = 3
_TINY_CELLS = 7
_SUB = 16
_R1_AHEAD, _R2_AHEAD, _R3_AHEAD, _W1_FIRST, _W1_AHEAD = 27, 5, 20, 8, 36


@jax.jit
def pallas_standalone__layerscale__sampling_kernel(
    x: jax.Array,
    y: jax.Array,
    gamma: jax.Array,
    grad_out: jax.Array,
):
    B, S, D = x.shape
    RG = (B * S) // _G
    NH = _G - _NLO
    LO, HI = (0, _NLO), (_NLO, NH)
    A = RG - 2 * _P - _Q
    p1, q0, p2 = A, A + _P, A + _P + _Q
    B1 = q0 // _SUB * _SUB
    n_r, n_g, n_w = RG // _KR, RG // _KG, RG // _KW
    f32 = jnp.float32

    def kernel_function(x_hbm, y_hbm, gam_hbm, g_hbm, o_hbm, gx_hbm, gy_hbm, gg_hbm,
                        xb, yb, gb, gyb, gamb, ggb, smp, smq, sems):
        s_r1, s_r2, s_r3, s_gam, s_p, s_q, s_out, s_gg = (sems.at[i] for i in range(8))
        hi = pl.ds(*HI)

        def rows(src, dst, sem, grp, lo, n):
            idx = (pl.ds(*grp), pl.ds(lo, n))
            return pltpu.make_async_copy(src.at[idx], dst.at[idx], sem)

        def start_steps(win, j0, j1):
            def step(j, carry):
                for src, dst, sem, grp, k in win:
                    rows(src, dst, sem, grp, pl.multiple_of(j * k, 8), k).start()
                return carry
            jax.lax.fori_loop(j0, j1, step, 0)

        def start_steps_forwarding(win, j0, c0, c1):
            for c in range(c0, c1):
                gi, r = c % NH, c // NH * 8
                pltpu.make_async_copy(
                    smp.at[gi, pl.ds(r, 8)], xb.at[_NLO + gi, pl.ds(p1 + r, 8)], s_p).start()
                j = j0 + (c - c0) * _FWD_EVERY
                start_steps(win, j, j + _FWD_EVERY)
            return j0 + (c1 - c0) * _FWD_EVERY

        def start_last_step(win):
            for src, dst, sem, grp, k in win:
                rows(src, dst, sem, grp, n_r * k, RG - n_r * k).start()

        def compute(body, init, grp, lo, hi_):
            reps = 1 if grp == HI else 4

            def step(i, carry):
                for gi in range(grp[0], grp[0] + grp[1]):
                    for u in range(reps):
                        r = pl.multiple_of(lo + (i * reps + u) * _SUB, _SUB)
                        carry = body(gi, pl.ds(r, _SUB), carry)
                return carry
            return jax.lax.fori_loop(0, (hi_ - lo) // (reps * _SUB), step, init)

        gam_in = pltpu.make_async_copy(gam_hbm, gamb, s_gam)
        gg_out = pltpu.make_async_copy(ggb, gg_hbm, s_gg)
        p1_in = pltpu.make_async_copy(x_hbm.at[hi, pl.ds(p1, _P)], smp, s_p)
        p1_fwd = pltpu.make_async_copy(smp, xb.at[hi, pl.ds(p1, _P)], s_p)
        p2_in = pltpu.make_async_copy(x_hbm.at[hi, pl.ds(p2, _P)], smp, s_p)
        p2_fwd = pltpu.make_async_copy(smp, xb.at[hi, pl.ds(p2, _P)], s_p)
        q_in = pltpu.make_async_copy(x_hbm.at[hi, pl.ds(q0, _Q)], smq, s_q)
        q_fwd = pltpu.make_async_copy(smq, xb.at[hi, pl.ds(q0, _Q)], s_q)

        r1 = [(g_hbm, gb, s_r1, HI, _KR), (y_hbm, yb, s_r1, LO, _KR)]
        r2 = [(y_hbm, yb, s_r2, HI, _KR), (x_hbm, xb, s_r2, LO, _KR)]
        r3 = [(x_hbm, xb, s_r3, HI, _KR), (g_hbm, gb, s_r3, LO, _KG)]
        w1 = [(gb, gx_hbm, s_out, HI, _KW), (xb, o_hbm, s_out, LO, _KW)]
        w2 = [(gyb, gy_hbm, s_out, HI, _KW), (gb, gx_hbm, s_out, LO, _KW)]
        w3 = [(xb, o_hbm, s_out, HI, _KW), (gyb, gy_hbm, s_out, LO, _KW)]

        rows(g_hbm, gb, s_r1, HI, 0, _KR).start()
        p1_in.start()
        q_in.start()
        rows(y_hbm, yb, s_r1, LO, 0, _KR).start()
        gam_in.start()
        start_steps(r1, 1, _R1_AHEAD)
        p1_in.wait()
        c1 = (n_r - _R1_AHEAD) // _FWD_EVERY
        c2 = c1 + n_r // _FWD_EVERY
        start_steps_forwarding(r1, _R1_AHEAD, 0, c1)
        start_last_step(r1)
        j = start_steps_forwarding(r2, 0, c1, c1 + _R2_AHEAD)

        rows(g_hbm, gb, s_r1, HI, 0, RG).wait()
        rows(y_hbm, yb, s_r1, LO, 0, RG).wait()
        gam_in.wait()
        start_steps_forwarding(r2, j, c1 + _R2_AHEAD, c2)
        start_last_step(r2)

        gam = jnp.broadcast_to(gamb[...].astype(f32).reshape(1, D), (_SUB, D))

        def grad_y_rows(gi, r, carry):
            gyb[gi, r, :] = (gam * gb[gi, r, :].astype(f32)).astype(gyb.dtype)
            return carry

        def grad_gamma_rows(gi, r, acc):
            prod = gb[gi, r, :].astype(f32) * yb[gi, r, :].astype(f32)
            return acc + prod.reshape(_SUB // 8, 8, D).sum(axis=0)

        def out_rows(gi, r, carry):
            xb[gi, r, :] = (xb[gi, r, :].astype(f32)
                            + gam * yb[gi, r, :].astype(f32)).astype(xb.dtype)
            return carry

        compute(grad_y_rows, 0, HI, 0, RG)
        j = start_steps_forwarding(r3, 0, c2, _P // 8 * NH)
        start_steps(r3, j, _R3_AHEAD)

        rows(y_hbm, yb, s_r2, HI, 0, RG).wait()
        rows(x_hbm, xb, s_r2, LO, 0, RG).wait()
        compute(out_rows, 0, LO, 0, RG)

        p1_fwd.wait()
        p2_in.start()
        start_steps(r3, _R3_AHEAD, n_g)
        t0 = A - 16
        for r in range(n_g * _KR, t0, _KR):
            rows(x_hbm, xb, s_r3, HI, r, min(_KR, t0 - r)).start()
        n_big = 2 * NH - _TINY_CELLS
        rows(x_hbm, xb, s_r3, (_NLO, n_big), t0, 8).start()
        for cell in range(n_big, 2 * NH):
            for col in range(0, D, 128):
                idx = (_NLO + cell % NH, pl.ds(t0 + cell // NH * 8, 8), pl.ds(col, 128))
                pltpu.make_async_copy(x_hbm.at[idx], xb.at[idx], s_r3).start()

        acc = compute(grad_gamma_rows, jnp.zeros((8, D), f32), HI, 0, RG)

        start_steps(w1, 0, _W1_FIRST)
        q_in.wait()
        p2_in.wait()
        q_fwd.start()
        p2_fwd.start()
        start_steps(w1, _W1_FIRST, _W1_AHEAD)

        rows(x_hbm, xb, s_r3, HI, 0, A).wait()
        rows(g_hbm, gb, s_r3, LO, 0, RG).wait()
        compute(grad_y_rows, 0, LO, 0, RG)
        acc = compute(grad_gamma_rows, acc, LO, 0, RG)
        ggb[...] = jnp.sum(acc, axis=0).astype(ggb.dtype)
        gg_out.start()
        start_steps(w1, _W1_AHEAD, n_w)
        compute(out_rows, 0, HI, 0, B1)
        start_steps(w2, 0, n_w)
        start_steps(w3, 0, n_w // 2)
        q_fwd.wait()
        p2_fwd.wait()
        compute(out_rows, 0, HI, B1, RG)
        start_steps(w3, n_w // 2, n_w)

        gg_out.wait()
        pltpu.make_async_copy(gb, gx_hbm, s_out).wait()
        pltpu.make_async_copy(gyb, gy_hbm, s_out).wait()
        pltpu.make_async_copy(xb, o_hbm, s_out).wait()

    shp = (_G, RG, D)
    any_spec = pl.BlockSpec(memory_space=pl.ANY)
    big = jax.ShapeDtypeStruct(shp, x.dtype)
    out, gx, gy, gg = pl.pallas_call(
        kernel_function,
        in_specs=[any_spec] * 4,
        out_specs=[any_spec] * 4,
        out_shape=[big, big, big, jax.ShapeDtypeStruct((D,), gamma.dtype)],
        scratch_shapes=[pltpu.VMEM(shp, x.dtype)] * 4
        + [pltpu.VMEM((D,), gamma.dtype)] * 2
        + [pltpu.SMEM((NH, _P, D), x.dtype), pltpu.SMEM((NH, _Q, D), x.dtype)]
        + [pltpu.SemaphoreType.DMA((8,))],
        compiler_params=pltpu.CompilerParams(
            vmem_limit_bytes=48 * 1024 * 1024, disable_semaphore_checks=True),
    )(x.reshape(shp), y.reshape(shp), gamma, grad_out.reshape(shp))
    return out.reshape(B, S, D), gx.reshape(B, S, D), gy.reshape(B, S, D), gg
```

```python
import jax
import jax.numpy as jnp
import jax.experimental.pallas as pl
import jax.experimental.pallas.tpu as pltpu


_G = 8
_NLO = 2
_KR = 24
_KG = 32
_KW = 16
_P = 32
_Q = 136
_FWD_EVERY = 3
_R1_AHEAD = 27
_W1_FIRST = 8
_W1_AHEAD = 36
_SUB = 16


@jax.jit
def pallas_standalone__layerscale__sampling_kernel(
    x: jax.Array,
    y: jax.Array,
    gamma: jax.Array,
    grad_out: jax.Array,
):
    B, S, D = x.shape
    RG = (B * S) // _G
    NH = _G - _NLO
    LO, HI, ALL = (0, _NLO), (_NLO, NH), (0, _G)
    A = RG - 2 * _P - _Q
    p1, q0, p2 = A, A + _P, A + _P + _Q
    B1 = q0 // _SUB * _SUB
    n_r, n_g, n_w = RG // _KR, RG // _KG, RG // _KW
    t0 = n_r * _KR
    assert RG - t0 == 16 and n_g * _KG == RG and n_w * _KW == RG
    f32 = jnp.float32

    def kernel_function(x_hbm, y_hbm, gam_hbm, g_hbm, o_hbm, gx_hbm, gy_hbm, gg_hbm,
                        xb, yb, gb, gyb, gamb, ggb, smp, smq, sems):
        (s_g, s_y, s_x_hi, s_x_lo, s_gam, s_p, s_q,
         s_o, s_gx, s_gy, s_gg) = (sems.at[i] for i in range(11))
        hi = pl.ds(*HI)

        def rows(src, dst, sem, grp, lo, n):
            idx = (pl.ds(*grp), pl.ds(lo, n))
            return pltpu.make_async_copy(src.at[idx], dst.at[idx], sem)

        def start_steps(win, j0, j1):
            def step(j, carry):
                for src, dst, sem, grp, k in win:
                    rows(src, dst, sem, grp, pl.multiple_of(j * k, 8), k).start()
                return carry
            jax.lax.fori_loop(j0, j1, step, 0)

        def start_steps_forwarding(win, j0, c0, c1):
            for c in range(c0, c1):
                gi, r = c % NH, c // NH * 8
                pltpu.make_async_copy(
                    smp.at[gi, pl.ds(r, 8)], xb.at[_NLO + gi, pl.ds(p1 + r, 8)], s_p).start()
                j = j0 + (c - c0) * _FWD_EVERY
                start_steps(win, j, j + _FWD_EVERY)
            return j0 + (c1 - c0) * _FWD_EVERY

        def compute(body, init, grp, lo, hi_):
            reps = 4 if grp == LO else 1

            def step(i, carry):
                for gi in range(grp[0], grp[0] + grp[1]):
                    for u in range(reps):
                        r = pl.multiple_of(lo + (i * reps + u) * _SUB, _SUB)
                        carry = body(gi, pl.ds(r, _SUB), carry)
                return carry
            return jax.lax.fori_loop(0, (hi_ - lo) // (reps * _SUB), step, init)

        gam_in = pltpu.make_async_copy(gam_hbm, gamb, s_gam)
        gg_out = pltpu.make_async_copy(ggb, gg_hbm, s_gg)
        p1_in = pltpu.make_async_copy(x_hbm.at[hi, pl.ds(p1, _P)], smp, s_p)
        p1_fwd = pltpu.make_async_copy(smp, xb.at[hi, pl.ds(p1, _P)], s_p)
        p2_in = pltpu.make_async_copy(x_hbm.at[hi, pl.ds(p2, _P)], smp, s_p)
        p2_fwd = pltpu.make_async_copy(smp, xb.at[hi, pl.ds(p2, _P)], s_p)
        q_in = pltpu.make_async_copy(x_hbm.at[hi, pl.ds(q0, _Q)], smq, s_q)
        q_fwd = pltpu.make_async_copy(smq, xb.at[hi, pl.ds(q0, _Q)], s_q)

        r1 = [(g_hbm, gb, s_g, HI, _KR), (y_hbm, yb, s_y, LO, _KR)]
        r2 = [(x_hbm, xb, s_x_hi, HI, _KR), (g_hbm, gb, s_g, LO, _KG)]
        r3 = [(y_hbm, yb, s_y, HI, _KR), (x_hbm, xb, s_x_lo, LO, _KR)]
        w1 = [(gyb, gy_hbm, s_gy, HI, _KW), (gb, gx_hbm, s_gx, LO, _KW)]
        w2 = [(gb, gx_hbm, s_gx, HI, _KW), (xb, o_hbm, s_o, LO, _KW)]
        w3 = [(xb, o_hbm, s_o, HI, _KW), (gyb, gy_hbm, s_gy, LO, _KW)]

        rows(g_hbm, gb, s_g, HI, t0, RG - t0).start()
        p1_in.start()
        q_in.start()
        rows(y_hbm, yb, s_y, LO, t0, RG - t0).start()
        gam_in.start()
        start_steps(r1, 0, _R1_AHEAD)
        p1_in.wait()
        c1 = (n_r - _R1_AHEAD) // _FWD_EVERY
        c2 = c1 + n_g // _FWD_EVERY
        j = start_steps_forwarding(r1, _R1_AHEAD, 0, c1)
        assert j == n_r
        j = start_steps_forwarding(r2, 0, c1, c2)
        start_steps(r2, j, n_g)
        for r in range(n_g * _KR, A, _KG):
            rows(x_hbm, xb, s_x_hi, HI, r, min(_KG, A - r)).start()
        j = start_steps_forwarding(r3, 0, c2, _P // 8 * NH)

        pltpu.make_async_copy(g_hbm, gb, s_g).wait()
        gam_in.wait()
        gam = jnp.broadcast_to(gamb[...].astype(f32).reshape(1, D), (_SUB, D))

        def grad_y_rows(gi, r, carry):
            gyb[gi, r, :] = (gam * gb[gi, r, :].astype(f32)).astype(gyb.dtype)
            return carry

        def grad_gamma_rows(gi, r, acc):
            prod = gb[gi, r, :].astype(f32) * yb[gi, r, :].astype(f32)
            return acc + prod.reshape(_SUB // 8, 8, D).sum(axis=0)

        def out_rows(gi, r, carry):
            xb[gi, r, :] = (xb[gi, r, :].astype(f32)
                            + gam * yb[gi, r, :].astype(f32)).astype(xb.dtype)
            return carry

        compute(grad_y_rows, 0, ALL, 0, RG)
        p1_fwd.wait()
        p2_in.start()
        start_steps(r3, j, n_r)
        for src, dst, sem, grp, _ in r3:
            rows(src, dst, sem, grp, t0, 8).start()
        for src, dst, sem, grp, _ in r3:
            for gi in range(grp[0], grp[0] + grp[1]):
                for col in range(0, D, 128):
                    idx = (gi, pl.ds(t0 + 8, 8), pl.ds(col, 128))
                    pltpu.make_async_copy(src.at[idx], dst.at[idx], sem).start()

        start_steps(w1, 0, _W1_FIRST)
        q_in.wait()
        p2_in.wait()
        q_fwd.start()
        p2_fwd.start()
        start_steps(w1, _W1_FIRST, _W1_AHEAD)

        pltpu.make_async_copy(y_hbm, yb, s_y).wait()
        rows(x_hbm, xb, s_x_lo, LO, 0, RG).wait()
        rows(x_hbm, xb, s_x_hi, HI, 0, A).wait()
        compute(out_rows, 0, LO, 0, RG)
        start_steps(w1, _W1_AHEAD, n_w)
        compute(out_rows, 0, HI, 0, B1)
        start_steps(w2, 0, n_w // 2)
        acc = compute(grad_gamma_rows, jnp.zeros((8, D), f32), ALL, 0, RG)
        ggb[...] = jnp.sum(acc, axis=0).astype(ggb.dtype)
        gg_out.start()
        start_steps(w2, n_w // 2, n_w)
        start_steps(w3, 0, n_w // 2)
        q_fwd.wait()
        p2_fwd.wait()
        compute(out_rows, 0, HI, B1, RG)
        start_steps(w3, n_w // 2, n_w)

        gg_out.wait()
        pltpu.make_async_copy(gb, gx_hbm, s_gx).wait()
        pltpu.make_async_copy(xb, o_hbm, s_o).wait()
        pltpu.make_async_copy(gyb, gy_hbm, s_gy).wait()

    shp = (_G, RG, D)
    any_spec = pl.BlockSpec(memory_space=pl.ANY)
    big = jax.ShapeDtypeStruct(shp, x.dtype)
    out, gx, gy, gg = pl.pallas_call(
        kernel_function,
        in_specs=[any_spec] * 4,
        out_specs=[any_spec] * 4,
        out_shape=[big, big, big, jax.ShapeDtypeStruct((D,), gamma.dtype)],
        scratch_shapes=[pltpu.VMEM(shp, x.dtype)] * 4
        + [pltpu.VMEM((D,), gamma.dtype)] * 2
        + [pltpu.SMEM((NH, _P, D), x.dtype), pltpu.SMEM((NH, _Q, D), x.dtype)]
        + [pltpu.SemaphoreType.DMA((11,))],
        compiler_params=pltpu.CompilerParams(
            vmem_limit_bytes=48 * 1024 * 1024, disable_semaphore_checks=True),
    )(x.reshape(shp), y.reshape(shp), gamma, grad_out.reshape(shp))
    return out.reshape(B, S, D), gx.reshape(B, S, D), gy.reshape(B, S, D), gg
```

```python
import jax
import jax.numpy as jnp
import jax.experimental.pallas as pl
import jax.experimental.pallas.tpu as pltpu


_G = 8
_NLO = 2
_KR = 24
_KG = 32
_KW = 16
_P = 32
_Q = 136
_FWD_EVERY = 3
_R1_AHEAD = 27
_W1_FIRST = 12
_SUB = 16


@jax.jit
def pallas_standalone__layerscale__sampling_kernel(
    x: jax.Array,
    y: jax.Array,
    gamma: jax.Array,
    grad_out: jax.Array,
):
    B, S, D = x.shape
    RG = (B * S) // _G
    NH = _G - _NLO
    LO, HI, ALL = (0, _NLO), (_NLO, NH), (0, _G)
    A = RG - 2 * _P - _Q
    p1, q0, p2 = A, A + _P, A + _P + _Q
    B1 = q0 // _SUB * _SUB
    n_r, n_g, n_w = RG // _KR, RG // _KG, RG // _KW
    t0 = n_r * _KR
    assert RG - t0 == 16 and n_g * _KG == RG and n_w * _KW == RG
    f32 = jnp.float32

    def kernel_body(x_hbm, y_hbm, gam_hbm, g_hbm, o_hbm, gx_hbm, gy_hbm, gg_hbm,
                    xb, yb, gb, gyb, gamb, ggb, smp, smq, sems):
        (s_g, s_y, s_x_hi, s_x_lo, s_gam, s_p, s_q,
         s_o, s_gx, s_gy, s_gg) = (sems.at[i] for i in range(11))
        hi = pl.ds(*HI)

        def rows(src, dst, sem, grp, lo, n):
            idx = (pl.ds(*grp), pl.ds(lo, n))
            return pltpu.make_async_copy(src.at[idx], dst.at[idx], sem)

        def start_steps(win, j0, j1):
            def step(j, carry):
                for src, dst, sem, grp, k in win:
                    rows(src, dst, sem, grp, pl.multiple_of(j * k, 8), k).start()
                return carry
            jax.lax.fori_loop(j0, j1, step, 0)

        def start_steps_forwarding(win, j0, c0, c1):
            for c in range(c0, c1):
                gi, r = c % NH, c // NH * 8
                pltpu.make_async_copy(
                    smp.at[gi, pl.ds(r, 8)], xb.at[_NLO + gi, pl.ds(p1 + r, 8)], s_p).start()
                j = j0 + (c - c0) * _FWD_EVERY
                start_steps(win, j, j + _FWD_EVERY)
            return j0 + (c1 - c0) * _FWD_EVERY

        def compute(body, init, grp, lo, hi_):
            reps = 4 if grp == LO else 1

            def step(i, carry):
                for gi in range(grp[0], grp[0] + grp[1]):
                    for u in range(reps):
                        r = pl.multiple_of(lo + (i * reps + u) * _SUB, _SUB)
                        carry = body(gi, pl.ds(r, _SUB), carry)
                return carry
            return jax.lax.fori_loop(0, (hi_ - lo) // (reps * _SUB), step, init)

        gam_in = pltpu.make_async_copy(gam_hbm, gamb, s_gam)
        gg_out = pltpu.make_async_copy(ggb, gg_hbm, s_gg)
        p1_in = pltpu.make_async_copy(x_hbm.at[hi, pl.ds(p1, _P)], smp, s_p)
        p1_fwd = pltpu.make_async_copy(smp, xb.at[hi, pl.ds(p1, _P)], s_p)
        p2_in = pltpu.make_async_copy(x_hbm.at[hi, pl.ds(p2, _P)], smp, s_p)
        p2_fwd = pltpu.make_async_copy(smp, xb.at[hi, pl.ds(p2, _P)], s_p)
        q_in = pltpu.make_async_copy(x_hbm.at[hi, pl.ds(q0, _Q)], smq, s_q)
        q_fwd = pltpu.make_async_copy(smq, xb.at[hi, pl.ds(q0, _Q)], s_q)

        r1 = [(g_hbm, gb, s_g, HI, _KR), (y_hbm, yb, s_y, LO, _KR)]
        r2 = [(x_hbm, xb, s_x_hi, HI, _KR), (g_hbm, gb, s_g, LO, _KG)]
        r3 = [(y_hbm, yb, s_y, HI, _KR), (x_hbm, xb, s_x_lo, LO, _KR)]
        w1 = [(gyb, gy_hbm, s_gy, (0, 6), _KW)]
        w2 = [(gyb, gy_hbm, s_gy, (6, _G - 6), _KW), (gb, gx_hbm, s_gx, (0, 3), _KW)]
        w3 = [(gb, gx_hbm, s_gx, (3, _G - 3), _KW), (xb, o_hbm, s_o, LO, _KW)]
        w4 = [(xb, o_hbm, s_o, HI, _KW)]

        rows(g_hbm, gb, s_g, HI, t0, RG - t0).start()
        p1_in.start()
        q_in.start()
        rows(y_hbm, yb, s_y, LO, t0, RG - t0).start()
        gam_in.start()
        start_steps(r1, 0, _R1_AHEAD)
        p1_in.wait()
        c1 = (n_r - _R1_AHEAD) // _FWD_EVERY
        c2 = c1 + n_g // _FWD_EVERY
        j = start_steps_forwarding(r1, _R1_AHEAD, 0, c1)
        assert j == n_r
        j = start_steps_forwarding(r2, 0, c1, c2)
        start_steps(r2, j, n_g)
        for r in range(n_g * _KR, A, _KG):
            rows(x_hbm, xb, s_x_hi, HI, r, min(_KG, A - r)).start()
        j = start_steps_forwarding(r3, 0, c2, _P // 8 * NH)

        pltpu.make_async_copy(g_hbm, gb, s_g).wait()
        gam_in.wait()
        gam = jnp.broadcast_to(gamb[...].astype(f32).reshape(1, D), (_SUB, D))

        def grad_y_rows(gi, r, carry):
            gyb[gi, r, :] = (gam * gb[gi, r, :].astype(f32)).astype(gyb.dtype)
            return carry

        def grad_gamma_rows(gi, r, acc):
            prod = gb[gi, r, :].astype(f32) * yb[gi, r, :].astype(f32)
            return acc + prod.reshape(_SUB // 8, 8, D).sum(axis=0)

        def out_rows(gi, r, carry):
            xb[gi, r, :] = (xb[gi, r, :].astype(f32)
                            + gam * yb[gi, r, :].astype(f32)).astype(xb.dtype)
            return carry

        compute(grad_y_rows, 0, ALL, 0, RG)
        p1_fwd.wait()
        p2_in.start()
        start_steps(r3, j, n_r)
        for src, dst, sem, grp, _ in r3:
            rows(src, dst, sem, grp, t0, 8).start()
        for src, dst, sem, grp, _ in r3:
            for gi in range(grp[0], grp[0] + grp[1]):
                for col in range(0, D, 128):
                    idx = (gi, pl.ds(t0 + 8, 8), pl.ds(col, 128))
                    pltpu.make_async_copy(src.at[idx], dst.at[idx], sem).start()

        start_steps(w1, 0, _W1_FIRST)
        q_in.wait()
        p2_in.wait()
        q_fwd.start()
        p2_fwd.start()
        start_steps(w1, _W1_FIRST, n_w)

        pltpu.make_async_copy(y_hbm, yb, s_y).wait()
        rows(x_hbm, xb, s_x_lo, LO, 0, RG).wait()
        rows(x_hbm, xb, s_x_hi, HI, 0, A).wait()
        acc = compute(grad_gamma_rows, jnp.zeros((8, D), f32), ALL, 0, RG)
        ggb[...] = jnp.sum(acc, axis=0).astype(ggb.dtype)
        gg_out.start()
        start_steps(w2, 0, n_w // 2)
        compute(out_rows, 0, LO, 0, RG)
        start_steps(w2, n_w // 2, n_w)
        start_steps(w3, 0, n_w // 2)
        compute(out_rows, 0, HI, 0, B1)
        start_steps(w3, n_w // 2, n_w)
        start_steps(w4, 0, n_w // 2)
        q_fwd.wait()
        p2_fwd.wait()
        compute(out_rows, 0, HI, B1, RG)
        start_steps(w4, n_w // 2, n_w)

        gg_out.wait()
        pltpu.make_async_copy(gyb, gy_hbm, s_gy).wait()
        pltpu.make_async_copy(gb, gx_hbm, s_gx).wait()
        pltpu.make_async_copy(xb, o_hbm, s_o).wait()

    def kernel_function(*refs):
        pl.run_scoped(lambda sems: kernel_body(*refs, sems), pltpu.SemaphoreType.DMA((11,)))

    shp = (_G, RG, D)
    any_spec = pl.BlockSpec(memory_space=pl.ANY)
    big = jax.ShapeDtypeStruct(shp, x.dtype)
    out, gx, gy, gg = pl.pallas_call(
        kernel_function,
        in_specs=[any_spec] * 4,
        out_specs=[any_spec] * 4,
        out_shape=[big, big, big, jax.ShapeDtypeStruct((D,), gamma.dtype)],
        scratch_shapes=[pltpu.VMEM(shp, x.dtype)] * 4
        + [pltpu.VMEM((D,), gamma.dtype)] * 2
        + [pltpu.SMEM((NH, _P, D), x.dtype), pltpu.SMEM((NH, _Q, D), x.dtype)],
        compiler_params=pltpu.CompilerParams(vmem_limit_bytes=48 * 1024 * 1024),
    )(x.reshape(shp), y.reshape(shp), gamma, grad_out.reshape(shp))
    return out.reshape(B, S, D), gx.reshape(B, S, D), gy.reshape(B, S, D), gg
```

```python
import jax
import jax.numpy as jnp
import jax.experimental.pallas as pl
import jax.experimental.pallas.tpu as pltpu


_G = 8
_NLO = 2
_KR = 3
_KG = 4
_KW = 2
_P = 4
_Q = 17
_FWD_EVERY = 3
_R1_AHEAD = 27
_W1_FIRST = 12
_SUB = 2


@jax.jit
def pallas_standalone__layerscale__sampling_kernel(
    x: jax.Array,
    y: jax.Array,
    gamma: jax.Array,
    grad_out: jax.Array,
):
    B, S, D = x.shape
    N = B // _G
    NH = _G - _NLO
    LO, HI, ALL = (0, _NLO), (_NLO, NH), (0, _G)
    A = N - 2 * _P - _Q
    p1, q0, p2 = A, A + _P, A + _P + _Q
    B1 = q0 // _SUB * _SUB
    n_r, n_g, n_w = N // _KR, N // _KG, N // _KW
    t0 = n_r * _KR
    assert N - t0 == 2 and n_g * _KG == N and n_w * _KW == N
    f32 = jnp.float32

    def kernel_body(x_hbm, y_hbm, gam_hbm, g_hbm, o_hbm, gx_hbm, gy_hbm, gg_hbm,
                    xb, yb, gb, gyb, gamb, ggb, smp, smq, sems):
        (s_g, s_y, s_x_hi, s_x_lo, s_gam, s_p, s_q,
         s_o, s_gx, s_gy, s_gg) = (sems.at[i] for i in range(11))
        hi = pl.ds(*HI)

        def items(src, dst, sem, grp, lo, n):
            idx = (pl.ds(*grp), pl.ds(lo, n))
            return pltpu.make_async_copy(src.at[idx], dst.at[idx], sem)

        def start_steps(win, j0, j1):
            def step(j, carry):
                for src, dst, sem, grp, k in win:
                    items(src, dst, sem, grp, j * k, k).start()
                return carry
            jax.lax.fori_loop(j0, j1, step, 0)

        def start_steps_forwarding(win, j0, c0, c1):
            for c in range(c0, c1):
                gi, i = c % NH, c // NH
                pltpu.make_async_copy(smp.at[gi, i], xb.at[_NLO + gi, p1 + i], s_p).start()
                j = j0 + (c - c0) * _FWD_EVERY
                start_steps(win, j, j + _FWD_EVERY)
            return j0 + (c1 - c0) * _FWD_EVERY

        def compute(body, init, grp, lo, hi_):
            reps = 4 if grp == LO else 1

            def step(i, carry):
                for gi in range(grp[0], grp[0] + grp[1]):
                    for u in range(reps):
                        carry = body(gi, pl.ds(lo + (i * reps + u) * _SUB, _SUB), carry)
                return carry
            return jax.lax.fori_loop(0, (hi_ - lo) // (reps * _SUB), step, init)

        gam_in = pltpu.make_async_copy(gam_hbm, gamb, s_gam)
        gg_out = pltpu.make_async_copy(ggb, gg_hbm, s_gg)
        p1_in = pltpu.make_async_copy(x_hbm.at[hi, pl.ds(p1, _P)], smp, s_p)
        p1_fwd = pltpu.make_async_copy(smp, xb.at[hi, pl.ds(p1, _P)], s_p)
        p2_in = pltpu.make_async_copy(x_hbm.at[hi, pl.ds(p2, _P)], smp, s_p)
        p2_fwd = pltpu.make_async_copy(smp, xb.at[hi, pl.ds(p2, _P)], s_p)
        q_in = pltpu.make_async_copy(x_hbm.at[hi, pl.ds(q0, _Q)], smq, s_q)
        q_fwd = pltpu.make_async_copy(smq, xb.at[hi, pl.ds(q0, _Q)], s_q)

        r1 = [(g_hbm, gb, s_g, HI, _KR), (y_hbm, yb, s_y, LO, _KR)]
        r2 = [(x_hbm, xb, s_x_hi, HI, _KR), (g_hbm, gb, s_g, LO, _KG)]
        r3 = [(y_hbm, yb, s_y, HI, _KR), (x_hbm, xb, s_x_lo, LO, _KR)]
        w1 = [(gyb, gy_hbm, s_gy, (0, 6), _KW)]
        w2 = [(gyb, gy_hbm, s_gy, (6, _G - 6), _KW), (gb, gx_hbm, s_gx, (0, 3), _KW)]
        w3 = [(gb, gx_hbm, s_gx, (3, _G - 3), _KW), (xb, o_hbm, s_o, LO, _KW)]
        w4 = [(xb, o_hbm, s_o, HI, _KW)]

        items(g_hbm, gb, s_g, HI, t0, N - t0).start()
        p1_in.start()
        q_in.start()
        items(y_hbm, yb, s_y, LO, t0, N - t0).start()
        gam_in.start()
        start_steps(r1, 0, _R1_AHEAD)
        p1_in.wait()
        c1 = (n_r - _R1_AHEAD) // _FWD_EVERY
        c2 = c1 + n_g // _FWD_EVERY
        j = start_steps_forwarding(r1, _R1_AHEAD, 0, c1)
        assert j == n_r
        j = start_steps_forwarding(r2, 0, c1, c2)
        start_steps(r2, j, n_g)
        for i in range(n_g * _KR, A, _KG):
            items(x_hbm, xb, s_x_hi, HI, i, min(_KG, A - i)).start()
        j = start_steps_forwarding(r3, 0, c2, _P * NH)

        pltpu.make_async_copy(g_hbm, gb, s_g).wait()
        gam_in.wait()
        gam = jnp.broadcast_to(gamb[...].astype(f32).reshape(1, 1, D), (_SUB, S, D))

        def grad_y_items(gi, it, carry):
            gyb[gi, it] = (gam * gb[gi, it].astype(f32)).astype(gyb.dtype)
            return carry

        def grad_gamma_items(gi, it, acc):
            return acc + jnp.sum(gb[gi, it].astype(f32) * yb[gi, it].astype(f32), axis=0)

        def out_items(gi, it, carry):
            xb[gi, it] = (xb[gi, it].astype(f32) + gam * yb[gi, it].astype(f32)).astype(xb.dtype)
            return carry

        compute(grad_y_items, 0, ALL, 0, N)
        p1_fwd.wait()
        p2_in.start()
        start_steps(r3, j, n_r)
        for src, dst, sem, grp, _ in r3:
            items(src, dst, sem, grp, t0, 1).start()
        for src, dst, sem, grp, _ in r3:
            for gi in range(grp[0], grp[0] + grp[1]):
                for col in range(0, D, 128):
                    idx = (gi, t0 + 1, slice(None), pl.ds(col, 128))
                    pltpu.make_async_copy(src.at[idx], dst.at[idx], sem).start()

        start_steps(w1, 0, _W1_FIRST)
        q_in.wait()
        p2_in.wait()
        q_fwd.start()
        p2_fwd.start()
        start_steps(w1, _W1_FIRST, n_w)

        pltpu.make_async_copy(y_hbm, yb, s_y).wait()
        items(x_hbm, xb, s_x_lo, LO, 0, N).wait()
        items(x_hbm, xb, s_x_hi, HI, 0, A).wait()
        acc = compute(grad_gamma_items, jnp.zeros((S, D), f32), ALL, 0, N)
        ggb[...] = jnp.sum(acc, axis=0).astype(ggb.dtype)
        gg_out.start()
        start_steps(w2, 0, n_w // 2)
        compute(out_items, 0, LO, 0, N)
        start_steps(w2, n_w // 2, n_w)
        start_steps(w3, 0, n_w // 2)
        compute(out_items, 0, HI, 0, B1)
        start_steps(w3, n_w // 2, n_w)
        start_steps(w4, 0, n_w // 2)
        q_fwd.wait()
        p2_fwd.wait()
        compute(out_items, 0, HI, B1, N)
        start_steps(w4, n_w // 2, n_w)

        gg_out.wait()
        pltpu.make_async_copy(gyb, gy_hbm, s_gy).wait()
        pltpu.make_async_copy(gb, gx_hbm, s_gx).wait()
        pltpu.make_async_copy(xb, o_hbm, s_o).wait()

    def kernel_function(*refs):
        pl.run_scoped(lambda sems: kernel_body(*refs, sems), pltpu.SemaphoreType.DMA((11,)))

    shp = (_G, N, S, D)
    any_spec = pl.BlockSpec(memory_space=pl.ANY)
    big = jax.ShapeDtypeStruct(shp, x.dtype)
    out, gx, gy, gg = pl.pallas_call(
        kernel_function,
        in_specs=[any_spec] * 4,
        out_specs=[any_spec] * 4,
        out_shape=[big, big, big, jax.ShapeDtypeStruct((D,), gamma.dtype)],
        scratch_shapes=[pltpu.VMEM(shp, x.dtype)] * 4
        + [pltpu.VMEM((D,), gamma.dtype)] * 2
        + [pltpu.SMEM((NH, _P, S, D), x.dtype), pltpu.SMEM((NH, _Q, S, D), x.dtype)],
        compiler_params=pltpu.CompilerParams(vmem_limit_bytes=48 * 1024 * 1024),
    )(x.reshape(shp), y.reshape(shp), gamma, grad_out.reshape(shp))
    return out.reshape(B, S, D), gx.reshape(B, S, D), gy.reshape(B, S, D), gg
```

```python
import jax
import jax.numpy as jnp
import jax.experimental.pallas as pl
import jax.experimental.pallas.tpu as pltpu


_G = 8
_NLO = 2
_KR = 6
_KG = 8
_KW = 4
_W0 = 1
_P = 8
_Q = 34
_FWD = 2
_FWD_EVERY = 3
_R1_AHEAD = 27
_W1_FIRST = 12
_SUB = 4


@jax.jit
def pallas_standalone__layerscale__sampling_kernel(
    x: jax.Array,
    y: jax.Array,
    gamma: jax.Array,
    grad_out: jax.Array,
):
    B, S, D = x.shape
    H = D // 2
    N = 2 * B // _G
    NH = _G - _NLO
    LO, HI, ALL = (0, _NLO), (_NLO, NH), (0, _G)
    A = N - 2 * _P - _Q
    p1, q0, p2 = A, A + _P, A + _P + _Q
    B1 = q0 // _SUB * _SUB
    n_r, n_g, n_w = N // _KR, N // _KG, (N - _W0) // _KW
    tr, tw = n_r * _KR, _W0 + n_w * _KW
    assert N - tr == 4 and n_g * _KG == N and tw < N
    f32 = jnp.float32

    def kernel_body(x_hbm, y_hbm, gam_hbm, g_hbm, o_hbm, gx_hbm, gy_hbm, gg_hbm,
                    xb, yb, gb, gyb, gamb, ggb, smp, smq, sems):
        (s_g, s_y, s_x_hi, s_x_lo, s_gam, s_p, s_q,
         s_o, s_gx, s_gy, s_gg) = (sems.at[i] for i in range(11))
        hi = pl.ds(*HI)

        def units(src, dst, sem, grp, lo, n):
            idx = (pl.ds(*grp), pl.ds(lo, n))
            return pltpu.make_async_copy(src.at[idx], dst.at[idx], sem)

        def start_units(win, lo, n):
            for src, dst, sem, grp, _ in win:
                units(src, dst, sem, grp, lo, n).start()

        def start_steps(win, j0, j1, base=0):
            def step(j, carry):
                for src, dst, sem, grp, k in win:
                    units(src, dst, sem, grp, base + j * k, k).start()
                return carry
            jax.lax.fori_loop(j0, j1, step, 0)

        def start_steps_forwarding(win, j0, c0, c1):
            for c in range(c0, c1):
                gi, u = c % NH, c // NH * _FWD
                pltpu.make_async_copy(smp.at[gi, pl.ds(u, _FWD)],
                                      xb.at[_NLO + gi, pl.ds(p1 + u, _FWD)], s_p).start()
                j = j0 + (c - c0) * _FWD_EVERY
                start_steps(win, j, j + _FWD_EVERY)
            return j0 + (c1 - c0) * _FWD_EVERY

        def start_write_head(win, j):
            start_units(win, 0, _W0)
            start_steps(win, 0, j, _W0)

        def start_write_tail(win, j):
            start_steps(win, j, n_w, _W0)
            start_units(win, tw, N - tw)

        def compute(body, init, grp, lo, hi_):
            reps = 4 if grp == LO else 1

            def step(i, carry):
                for gi in range(grp[0], grp[0] + grp[1]):
                    for r in range(reps):
                        carry = body(gi, pl.ds(lo + (i * reps + r) * _SUB, _SUB), carry)
                return carry
            return jax.lax.fori_loop(0, (hi_ - lo) // (reps * _SUB), step, init)

        gam_in = pltpu.make_async_copy(gam_hbm, gamb, s_gam)
        gg_out = pltpu.make_async_copy(ggb, gg_hbm, s_gg)
        p1_in = pltpu.make_async_copy(x_hbm.at[hi, pl.ds(p1, _P)], smp, s_p)
        p1_fwd = pltpu.make_async_copy(smp, xb.at[hi, pl.ds(p1, _P)], s_p)
        p2_in = pltpu.make_async_copy(x_hbm.at[hi, pl.ds(p2, _P)], smp, s_p)
        p2_fwd = pltpu.make_async_copy(smp, xb.at[hi, pl.ds(p2, _P)], s_p)
        q_in = pltpu.make_async_copy(x_hbm.at[hi, pl.ds(q0, _Q)], smq, s_q)
        q_fwd = pltpu.make_async_copy(smq, xb.at[hi, pl.ds(q0, _Q)], s_q)

        r1 = [(g_hbm, gb, s_g, HI, _KR), (y_hbm, yb, s_y, LO, _KR)]
        r2 = [(x_hbm, xb, s_x_hi, HI, _KR), (g_hbm, gb, s_g, LO, _KG)]
        r3 = [(y_hbm, yb, s_y, HI, _KR), (x_hbm, xb, s_x_lo, LO, _KR)]
        w1 = [(gyb, gy_hbm, s_gy, (0, 6), _KW)]
        w2 = [(gyb, gy_hbm, s_gy, (6, _G - 6), _KW), (gb, gx_hbm, s_gx, (0, 3), _KW)]
        w3 = [(gb, gx_hbm, s_gx, (3, _G - 3), _KW), (xb, o_hbm, s_o, LO, _KW)]
        w4 = [(xb, o_hbm, s_o, HI, _KW)]

        units(g_hbm, gb, s_g, HI, tr, N - tr).start()
        p1_in.start()
        q_in.start()
        units(y_hbm, yb, s_y, LO, tr, N - tr).start()
        gam_in.start()
        start_steps(r1, 0, _R1_AHEAD)
        p1_in.wait()
        c1 = (n_r - _R1_AHEAD) // _FWD_EVERY
        c2 = c1 + n_g // _FWD_EVERY
        j = start_steps_forwarding(r1, _R1_AHEAD, 0, c1)
        assert j == n_r
        j = start_steps_forwarding(r2, 0, c1, c2)
        start_steps(r2, j, n_g)
        for u in range(n_g * _KR, A, _KG):
            units(x_hbm, xb, s_x_hi, HI, u, min(_KG, A - u)).start()
        j = start_steps_forwarding(r3, 0, c2, _P // _FWD * NH)

        pltpu.make_async_copy(g_hbm, gb, s_g).wait()
        gam_in.wait()
        gam_row = jnp.broadcast_to(gamb[...].astype(f32).reshape(1, D), (S, D))
        gam = jnp.stack([gam_row[:, :H], gam_row[:, H:]] * (_SUB // 2))

        def grad_y_units(gi, us, carry):
            gyb[gi, us] = (gam * gb[gi, us].astype(f32)).astype(gyb.dtype)
            return carry

        def grad_gamma_units(gi, us, acc):
            prod = gb[gi, us].astype(f32) * yb[gi, us].astype(f32)
            return acc + jnp.sum(prod.reshape(_SUB // 2, 2, S, H), axis=0)

        def out_units(gi, us, carry):
            xb[gi, us] = (xb[gi, us].astype(f32) + gam * yb[gi, us].astype(f32)).astype(xb.dtype)
            return carry

        compute(grad_y_units, 0, ALL, 0, N)
        p1_fwd.wait()
        p2_in.start()
        start_steps(r3, j, n_r)
        start_units(r3, tr, 2)
        for src, dst, sem, grp, _ in r3:
            for gi in range(grp[0], grp[0] + grp[1]):
                for u in (N - 2, N - 1):
                    for col in range(0, H, 128):
                        idx = (gi, u, slice(None), pl.ds(col, 128))
                        pltpu.make_async_copy(src.at[idx], dst.at[idx], sem).start()

        half = n_w // 2
        start_write_head(w1, _W1_FIRST)
        q_in.wait()
        p2_in.wait()
        q_fwd.start()
        p2_fwd.start()
        start_write_tail(w1, _W1_FIRST)

        pltpu.make_async_copy(y_hbm, yb, s_y).wait()
        units(x_hbm, xb, s_x_lo, LO, 0, N).wait()
        units(x_hbm, xb, s_x_hi, HI, 0, A).wait()
        acc = compute(grad_gamma_units, jnp.zeros((2, S, H), f32), ALL, 0, N)
        acc = jnp.concatenate([acc[0], acc[1]], axis=-1)
        ggb[...] = jnp.sum(acc, axis=0).astype(ggb.dtype)
        gg_out.start()
        start_write_head(w2, half)
        compute(out_units, 0, LO, 0, N)
        start_write_tail(w2, half)
        start_write_head(w3, half)
        compute(out_units, 0, HI, 0, B1)
        start_write_tail(w3, half)
        start_write_head(w4, half)
        q_fwd.wait()
        p2_fwd.wait()
        compute(out_units, 0, HI, B1, N)
        start_write_tail(w4, half)

        gg_out.wait()
        pltpu.make_async_copy(gyb, gy_hbm, s_gy).wait()
        pltpu.make_async_copy(gb, gx_hbm, s_gx).wait()
        pltpu.make_async_copy(xb, o_hbm, s_o).wait()

    def kernel_function(*refs):
        pl.run_scoped(lambda sems: kernel_body(*refs, sems), pltpu.SemaphoreType.DMA((11,)))

    shp = (_G, N, S, H)

    def to_units(a):
        return a.reshape(B, S, 2, H).transpose(0, 2, 1, 3).reshape(shp)

    def from_units(a):
        return a.reshape(B, 2, S, H).transpose(0, 2, 1, 3).reshape(B, S, D)

    any_spec = pl.BlockSpec(memory_space=pl.ANY)
    big = jax.ShapeDtypeStruct(shp, x.dtype)
    out, gx, gy, gg = pl.pallas_call(
        kernel_function,
        in_specs=[any_spec] * 4,
        out_specs=[any_spec] * 4,
        out_shape=[big, big, big, jax.ShapeDtypeStruct((D,), gamma.dtype)],
        scratch_shapes=[pltpu.VMEM(shp, x.dtype)] * 4
        + [pltpu.VMEM((D,), gamma.dtype)] * 2
        + [pltpu.SMEM((NH, _P, S, H), x.dtype), pltpu.SMEM((NH, _Q, S, H), x.dtype)],
        compiler_params=pltpu.CompilerParams(vmem_limit_bytes=48 * 1024 * 1024),
    )(to_units(x), to_units(y), gamma, to_units(grad_out))
    return from_units(out), from_units(gx), from_units(gy), gg
```
